```python
import os as _os
_os.environ.setdefault("JAX_PLATFORMS", "cpu")
import jax
import jax.numpy as jnp

def _softmax(x, axis=-1):
    return jax.nn.softmax(x, axis=axis)
def _gelu(x):
    return jax.nn.gelu(x, approximate=True)
def _silu(x):
    return jax.nn.silu(x)
def _sigmoid(x):
    return jax.nn.sigmoid(x)
def _layernorm(x, axis=-1, eps=1e-5):
    m = jnp.mean(x, axis=axis, keepdims=True)
    v = jnp.var(x, axis=axis, keepdims=True)
    return (x - m) / jnp.sqrt(v + eps)
def _scatter_add(tgt, idx, src, axis=0):
    return tgt.at[idx].add(src)
def _segment_sum(src, seg, n):
    return jax.ops.segment_sum(src, seg, n)
class _Rng:
    def __init__(self, key):
        self._k = key
    def _next(self):
        self._k, sub = jax.random.split(self._k)
        return sub
    def normal(self, shape):
        return jax.random.normal(self._next(), shape, dtype=jnp.bfloat16)
    def randint(self, lo, hi, shape):
        return jax.random.randint(self._next(), shape, lo, hi, dtype=jnp.int32)
    def uniform(self, shape, lo=0.0, hi=1.0):
        return jax.random.uniform(self._next(), shape, jnp.bfloat16, lo, hi)
    def permutation(self, n):
        return jax.random.permutation(self._next(), n)


kernel_name = 'sequential_preLN__linear_attn_block__dense_activation_squared_relu__prompt'

def setup_inputs():
    _rng = _Rng(jax.random.key(int.from_bytes(__import__("os").urandom(4), "little")))
    _w = (lambda a: (lambda t: t.astype(jnp.bfloat16) if jnp.issubdtype(t.dtype, jnp.floating) else t)(jnp.asarray(a)))
    def _A_setup():
        B, S, D = 1, 2048, 576
        return {
            "x": _w((lambda *s: _rng.normal(s) * 0.05)(B, S, D)),
            "wqkv": _w((lambda *s: _rng.normal(s) * 0.1)(D, 3 * D)),
            "wo": _w((lambda *s: _rng.normal(s) * 0.05)(D, D)),
        }
    _A_in = _A_setup()

    def _B_setup():
        B, S, D, F = 1, 2048, 576, 4608
        return {
            "x": _w((lambda *s: _rng.normal(s) * 0.05)(B, S, D)),
            "w1": _w((lambda *s: _rng.normal(s) * 0.05)(D, F)),
            "b1": _w((lambda *s: _rng.normal(s) * 0.05)(F)),
            "w2": _w((lambda *s: _rng.normal(s) * 0.05)(F, D)),
            "b2": _w((lambda *s: _rng.normal(s) * 0.05)(D)),
        }
    _B_in = _B_setup()

    return {
        "A_x": _A_in["x"],
        "A_wqkv": _A_in["wqkv"],
        "A_wo": _A_in["wo"],
        "B_x": _B_in["x"],
        "B_w1": _B_in["w1"],
        "B_b1": _B_in["b1"],
        "B_w2": _B_in["w2"],
        "B_b2": _B_in["b2"],
    }

def reference(A_x, A_wqkv, A_wo, B_x, B_w1, B_b1, B_w2, B_b2):
    def _A_ref(x, wqkv, wo):
        B, S, D = x.shape
        H = 32; Dh = D // H
        qkv = (lambda x, *d: x.transpose(*d))((x @ wqkv).reshape(B, S, 3, H, Dh), 2, 0, 3, 1, 4)
        q, k, v = qkv[0], qkv[1], qkv[2]
        phi = lambda t: jnp.where(t > 0, t + 1, jnp.exp(t)) + 1e-6
        pq, pk = phi(q), phi(k)
        kv = jnp.einsum("bhsd,bhse->bhde", pk, v)
        z = jnp.einsum("bhsd->bhd", pk)
        num = jnp.einsum("bhqd,bhde->bhqe", pq, kv)
        den = jnp.einsum("bhqd,bhd->bhq", pq, z)[..., None] + 1e-6
        o = num / den
        return (lambda x, *d: x.transpose(*d))(o, 0, 2, 1, 3).reshape(B, S, D) @ wo

    def _B_ref(x, w1, b1, w2, b2):
        h = jnp.einsum("bsd,df->bsf", x, w1) + b1
        zero = jnp.zeros_like(h)
        r = jnp.where(h > zero, h, zero)
        h = r * r
        out = jnp.einsum("bsf,fd->bsd", h, w2) + b2
        return out

    x = A_x
    h = x + _A_ref(_layernorm(x, axis=-1), A_wqkv, A_wo)
    h2 = h + _B_ref(_layernorm(h, axis=-1), B_w1, B_b1, B_w2, B_b2)
    return h2
```

```python
import functools
import jax
import jax.numpy as jnp
import jax.experimental.pallas as pl
import jax.experimental.pallas.tpu as pltpu

S, D, F, H, DH = 2048, 576, 4608, 32, 18
DP = 640
TM = 512
FC = 512
MLP = 'T'
NS = S // TM
NFC = F // FC
EPS = 1e-5
bf16 = jnp.bfloat16
f32 = jnp.float32
NT = (((1,), (1,)), ((), ()))


def _ln0(x):
    m = jnp.mean(x, axis=0, keepdims=True)
    xc = x - m
    v = jnp.mean(xc * xc, axis=0, keepdims=True)
    return xc * jax.lax.rsqrt(v + EPS)


def _phi(t):
    return jnp.where(t > 0, t + 1.0, jnp.exp(jnp.minimum(t, 0.0))) + 1e-6


def _head(idx):
    return sum((idx >= DH * j).astype(jnp.int32) for j in range(1, H))


def _kernel(x_ref, wqkv_ref, b1_ref, b2_ref, wo_hbm, w1_hbm, w2_hbm, o_ref,
            wqkT, wo_v, w1_v, w1T, w2_v, pq_s, g_acc, wpT, zbd, b1c, b2c, sems):
    step = pl.program_id(0)

    def copies():
        return [pltpu.make_async_copy(wo_hbm, wo_v, sems.at[0]),
                pltpu.make_async_copy(w1_hbm, w1_v, sems.at[1]),
                pltpu.make_async_copy(w2_hbm, w2_v, sems.at[2])]

    @pl.when(step == 0)
    def _():
        for c in copies():
            c.start()
        wqkT[...] = wqkv_ref[:, :2 * D].T
        g_acc[...] = jnp.zeros(g_acc.shape, f32)

    @pl.when(step < NS)
    def _():
        x = x_ref[...].astype(f32)
        xn = _ln0(x).astype(bf16)
        qk = jnp.dot(wqkT[...], xn, preferred_element_type=f32)
        col0 = pl.multiple_of(step * TM, TM)
        pq_s[:, pl.ds(col0, TM)] = _phi(qk[:D, :]).astype(bf16)
        pk = _phi(qk[D:, :]).astype(bf16)
        xe = jnp.concatenate([xn, jnp.ones((DP - D, TM), bf16)], axis=0)
        g_acc[...] += jax.lax.dot_general(pk, xe, NT, preferred_element_type=f32)

    @pl.when(step == NS - 1)
    def _():
        for c in copies():
            c.wait()
        if MLP == 'T':
            for c in range(NFC):
                w1T[c * FC:(c + 1) * FC, :] = w1_v[:, c * FC:(c + 1) * FC].T
            b1c[...] = jnp.broadcast_to(b1_ref[...].astype(f32), (128, F)).T
        b2c[...] = jnp.broadcast_to(b2_ref[...].astype(f32), (128, D)).T
        g = g_acc[...]
        kv = jnp.dot(g[:, :D].astype(bf16), wqkv_ref[:, 2 * D:], preferred_element_type=f32)
        r = jax.lax.broadcasted_iota(jnp.int32, (D, D), 0)
        c = jax.lax.broadcasted_iota(jnp.int32, (D, D), 1)
        mask = _head(r) == _head(c)
        kvbd = jnp.where(mask, kv, 0.0).astype(bf16)
        wp = jnp.dot(kvbd, wo_v[...], preferred_element_type=f32)
        wpT[...] = wp.T.astype(bf16)
        z = g[:, D:D + 1]
        zbd[...] = jnp.where(mask, jnp.broadcast_to(z, (D, D)), 0.0).T.astype(bf16)

    @pl.when(step >= NS)
    def _():
        col0 = pl.multiple_of((step - NS) * TM, TM)
        x = x_ref[...].astype(f32)
        pq = pq_s[:, pl.ds(col0, TM)]
        den = jnp.dot(zbd[...], pq, preferred_element_type=f32) + 1e-6
        pqn = (pq.astype(f32) / den).astype(bf16)
        h = x + jnp.dot(wpT[...], pqn, preferred_element_type=f32)
        hn = _ln0(h).astype(bf16)
        acc = h + jnp.concatenate([b2c[...]] * (TM // 128), axis=1)
        if MLP == 'T':
            for c in range(NFC):
                a = jnp.dot(w1T[c * FC:(c + 1) * FC, :], hn, preferred_element_type=f32)
                a = a + jnp.concatenate([b1c[c * FC:(c + 1) * FC, :]] * (TM // 128), axis=1)
                a = jnp.maximum(a, 0.0)
                a = (a * a).astype(bf16)
                acc = acc + jnp.dot(w2_v[:, c * FC:(c + 1) * FC], a, preferred_element_type=f32)
        else:
            hnN = hn.T
            for c in range(NFC):
                a = jnp.dot(hnN, w1_v[:, c * FC:(c + 1) * FC], preferred_element_type=f32)
                a = a + b1_ref[:, c * FC:(c + 1) * FC].astype(f32)
                a = jnp.maximum(a, 0.0)
                a = (a * a).astype(bf16)
                acc = acc + jax.lax.dot_general(w2_v[:, c * FC:(c + 1) * FC], a, NT,
                                                preferred_element_type=f32)
        o_ref[...] = acc.astype(o_ref.dtype)


@jax.jit
def pallas_sequential_preLN__linear_attn_block__dense_activation_squared_relu__prompt_kernel(
    A_x, A_wqkv, A_wo, B_x, B_w1, B_b1, B_w2, B_b2):
    xT = jnp.swapaxes(A_x, 1, 2).reshape(D, S)
    w2T = B_w2.T
    b1 = B_b1.reshape(1, F)
    b2 = B_b2.reshape(1, D)
    out = pl.pallas_call(
        _kernel,
        grid=(2 * NS,),
        in_specs=[
            pl.BlockSpec((D, TM), lambda i: (0, i % NS)),
            pl.BlockSpec((D, 3 * D), lambda i: (0, 0)),
            pl.BlockSpec((1, F), lambda i: (0, 0)),
            pl.BlockSpec((1, D), lambda i: (0, 0)),
            pl.BlockSpec(memory_space=pl.ANY),
            pl.BlockSpec(memory_space=pl.ANY),
            pl.BlockSpec(memory_space=pl.ANY),
        ],
        out_specs=pl.BlockSpec((D, TM), lambda i: (0, jnp.maximum(i - NS, 0))),
        out_shape=jax.ShapeDtypeStruct((D, S), bf16),
        scratch_shapes=[
            pltpu.VMEM((2 * D, D), bf16),
            pltpu.VMEM((D, D), bf16),
            pltpu.VMEM((D, F), bf16),
            pltpu.VMEM((F, D), bf16),
            pltpu.VMEM((D, F), bf16),
            pltpu.VMEM((D, S), bf16),
            pltpu.VMEM((D, DP), f32),
            pltpu.VMEM((D, D), bf16),
            pltpu.VMEM((D, D), bf16),
            pltpu.VMEM((F, 128), f32),
            pltpu.VMEM((D, 128), f32),
            pltpu.SemaphoreType.DMA((3,)),
        ],
        compiler_params=pltpu.CompilerParams(
            dimension_semantics=("arbitrary",),
            vmem_limit_bytes=100 * 1024 * 1024),
    )(xT, A_wqkv, b1, b2, A_wo, B_w1, w2T)
    return jnp.swapaxes(out.reshape(1, D, S), 1, 2)
```

```python
import functools
import jax
import jax.numpy as jnp
import jax.experimental.pallas as pl
import jax.experimental.pallas.tpu as pltpu

S, D, F, H, DH = 2048, 576, 4608, 32, 18
DP = 640
TM = 512
FC = 512
NS = S // TM
NFC = F // FC
EPS = 1e-5
bf16 = jnp.bfloat16
f32 = jnp.float32
NT = (((1,), (1,)), ((), ()))

BANDS = []
for _j in range(5):
    _lo, _hi = 128 * _j, min(128 * (_j + 1), D)
    _r0 = (_lo // DH) * DH
    _r1 = ((_hi - 1) // DH + 1) * DH
    BANDS.append((_lo, _hi, (_r0 // 16) * 16, -(-_r1 // 16) * 16))


def _band_assemble(parts):
    pieces = []
    cur = 0
    for j, (_, _, r0, r1) in enumerate(BANDS):
        p = parts[j]
        nxt = BANDS[j + 1][2] if j + 1 < len(BANDS) else D
        a = p[cur - r0:nxt - r0]
        pieces.append(a)
        if j + 1 < len(BANDS):
            ov = p[nxt - r0:r1 - r0] + parts[j + 1][:r1 - nxt]
            pieces.append(ov)
            cur = r1
    return jnp.concatenate(pieces, axis=0)


def _ln0(x):
    m = jnp.mean(x, axis=0, keepdims=True)
    xc = x - m
    v = jnp.mean(xc * xc, axis=0, keepdims=True)
    return xc * jax.lax.rsqrt(v + EPS)


def _phi(t):
    return jnp.where(t > 0, t + 1.0, jnp.exp(jnp.minimum(t, 0.0))) + 1e-6


def _head(idx):
    return sum((idx >= DH * j).astype(jnp.int32) for j in range(1, H))


def _kernel(x_hbm, wqkv_hbm, b1_hbm, b2_hbm, wo_hbm, w1_hbm, w2_hbm, o_ref,
            x_v, wqk_v, wv_v, wqkT, wo_v, w1_v, w1T, w2_v, b1_v, b2_v,
            pq_s, g_acc, wpT, zbd, b1c, b2c, sems):
    step = pl.program_id(0)

    def x_copy(i):
        return pltpu.make_async_copy(x_hbm.at[:, pl.ds(i * TM, TM)],
                                     x_v.at[:, pl.ds(i * TM, TM)], sems.at[i])

    wqk_copy = pltpu.make_async_copy(wqkv_hbm.at[:, pl.ds(0, 2 * D)], wqk_v, sems.at[NS])
    w1_copies = [pltpu.make_async_copy(w1_hbm, w1_v, sems.at[NS + 1]),
                 pltpu.make_async_copy(b1_hbm, b1_v, sems.at[NS + 2]),
                 pltpu.make_async_copy(b2_hbm, b2_v, sems.at[NS + 3])]
    late_copies = [pltpu.make_async_copy(wqkv_hbm.at[:, pl.ds(2 * D, D)], wv_v, sems.at[NS + 4]),
                   pltpu.make_async_copy(wo_hbm, wo_v, sems.at[NS + 5])]
    w2_copy = pltpu.make_async_copy(w2_hbm, w2_v, sems.at[NS + 6])

    @pl.when(step == 0)
    def _():
        x_copy(0).start()
        wqk_copy.start()
        for k in range(1, NS):
            x_copy(k).start()
        for c in w1_copies + late_copies + [w2_copy]:
            c.start()
        wqk_copy.wait()
        wqkT[...] = wqk_v[...].T
        g_acc[...] = jnp.zeros(g_acc.shape, f32)

    def phase1(prep):
        col0 = pl.multiple_of(step * TM, TM)
        pltpu.make_async_copy(x_hbm.at[:, pl.ds(col0, TM)],
                              x_v.at[:, pl.ds(col0, TM)], sems.at[step]).wait()
        if prep:
            for c in w1_copies:
                c.wait()
            for c in range(NFC):
                w1T[c * FC:(c + 1) * FC, :] = w1_v[:, c * FC:(c + 1) * FC].T
            b1c[...] = jnp.broadcast_to(b1_v[...].astype(f32).reshape(1, F), (128, F)).T
            b2c[...] = jnp.broadcast_to(b2_v[...].astype(f32).reshape(1, D), (128, D)).T
        x = x_v[:, pl.ds(col0, TM)].astype(f32)
        xn = _ln0(x).astype(bf16)
        qk = jnp.dot(wqkT[...], xn, preferred_element_type=f32)
        pq_s[:, pl.ds(col0, TM)] = _phi(qk[:D, :]).astype(bf16)
        pk = _phi(qk[D:, :]).astype(bf16)
        xe = jnp.concatenate([xn, jnp.ones((DP - D, TM), bf16)], axis=0)
        g_acc[...] += jax.lax.dot_general(pk, xe, NT, preferred_element_type=f32)

    @pl.when(jnp.logical_and(step < NS, step != NS - 2))
    def _():
        phase1(False)

    @pl.when(step == NS - 2)
    def _():
        phase1(True)

    @pl.when(step == NS - 1)
    def _():
        for c in late_copies:
            c.wait()
        wp_parts = []
        for (lo, hi, r0, r1) in BANDS:
            g = g_acc[r0:r1, :]
            kv = jnp.dot(g[:, :D].astype(bf16), wv_v[:, lo:hi], preferred_element_type=f32)
            r = jax.lax.broadcasted_iota(jnp.int32, (r1 - r0, hi - lo), 0) + r0
            c = jax.lax.broadcasted_iota(jnp.int32, (r1 - r0, hi - lo), 1) + lo
            mask = _head(r) == _head(c)
            kvbd = jnp.where(mask, kv, 0.0).astype(bf16)
            wp_parts.append(jnp.dot(kvbd, wo_v[lo:hi, :], preferred_element_type=f32))
            zc = g_acc[lo:hi, D:D + 1]
            zrow = jnp.broadcast_to(zc, (hi - lo, r1 - r0)).T
            zbd[r0:r1, lo:hi] = jnp.where(mask, zrow, 0.0).astype(bf16)
        wpT[...] = _band_assemble(wp_parts).T.astype(bf16)

    @pl.when(step >= NS)
    def _():
        @pl.when(step == NS)
        def _():
            w2_copy.wait()
        col0 = pl.multiple_of((step - NS) * TM, TM)
        x = x_v[:, pl.ds(col0, TM)].astype(f32)
        pq = pq_s[:, pl.ds(col0, TM)]
        den = _band_assemble([
            jnp.dot(zbd[r0:r1, lo:hi], pq[lo:hi, :], preferred_element_type=f32)
            for (lo, hi, r0, r1) in BANDS]) + 1e-6
        pqn = (pq.astype(f32) / den).astype(bf16)
        h = x + jnp.dot(wpT[...], pqn, preferred_element_type=f32)
        hn = _ln0(h).astype(bf16)
        acc = h + jnp.concatenate([b2c[...]] * (TM // 128), axis=1)
        for c in range(NFC):
            a = jnp.dot(w1T[c * FC:(c + 1) * FC, :], hn, preferred_element_type=f32)
            a = a + jnp.concatenate([b1c[c * FC:(c + 1) * FC, :]] * (TM // 128), axis=1)
            a = jnp.maximum(a, 0.0)
            a = (a * a).astype(bf16)
            acc = acc + jnp.dot(w2_v[:, c * FC:(c + 1) * FC], a, preferred_element_type=f32)
        o_ref[...] = acc.astype(o_ref.dtype)


@jax.jit
def pallas_sequential_preLN__linear_attn_block__dense_activation_squared_relu__prompt_kernel(
    A_x, A_wqkv, A_wo, B_x, B_w1, B_b1, B_w2, B_b2):
    xT = jnp.swapaxes(A_x, 1, 2).reshape(D, S)
    w2T = B_w2.T
    out = pl.pallas_call(
        _kernel,
        grid=(2 * NS,),
        in_specs=[pl.BlockSpec(memory_space=pl.ANY)] * 7,
        out_specs=pl.BlockSpec((D, TM), lambda i: (0, jnp.maximum(i - NS, 0))),
        out_shape=jax.ShapeDtypeStruct((D, S), bf16),
        scratch_shapes=[
            pltpu.VMEM((D, S), bf16),
            pltpu.VMEM((D, 2 * D), bf16),
            pltpu.VMEM((D, D), bf16),
            pltpu.VMEM((2 * D, D), bf16),
            pltpu.VMEM((D, D), bf16),
            pltpu.VMEM((D, F), bf16),
            pltpu.VMEM((F, D), bf16),
            pltpu.VMEM((D, F), bf16),
            pltpu.VMEM((F,), bf16),
            pltpu.VMEM((D,), bf16),
            pltpu.VMEM((D, S), bf16),
            pltpu.VMEM((D, DP), f32),
            pltpu.VMEM((D, D), bf16),
            pltpu.VMEM((D, D), bf16),
            pltpu.VMEM((F, 128), f32),
            pltpu.VMEM((D, 128), f32),
            pltpu.SemaphoreType.DMA((NS + 7,)),
        ],
        compiler_params=pltpu.CompilerParams(
            dimension_semantics=("arbitrary",),
            vmem_limit_bytes=100 * 1024 * 1024),
    )(xT, A_wqkv, B_b1, B_b2, A_wo, B_w1, w2T)
    return jnp.swapaxes(out.reshape(1, D, S), 1, 2)
```

```python
import jax
import jax.numpy as jnp
import jax.experimental.pallas as pl
import jax.experimental.pallas.tpu as pltpu

S, D, F, H, DH = 2048, 576, 4608, 32, 18
DP = 640
TM = 512
FC = 768
NS = S // TM
F2 = F // 2
D2 = D // 2
KM = 256
N2 = TM // 2
NFC = F2 // FC
WQ = 640
A2_SLOTS = (0, 1, 4, 5, 6)
RB = 16
EPS = 1e-5
bf16 = jnp.bfloat16
f32 = jnp.float32
NT = (((1,), (1,)), ((), ()))

BANDS = []
for _j in range(5):
    _lo, _hi = 128 * _j, min(128 * (_j + 1), D)
    _r0 = (_lo // DH) * DH
    _r1 = ((_hi - 1) // DH + 1) * DH
    BANDS.append((_lo, _hi, (_r0 // 16) * 16, -(-_r1 // 16) * 16))


def _band_assemble(parts):
    pieces = []
    cur = 0
    for j, (_, _, r0, r1) in enumerate(BANDS):
        p = parts[j]
        nxt = BANDS[j + 1][2] if j + 1 < len(BANDS) else D
        pieces.append(p[cur - r0:nxt - r0])
        if j + 1 < len(BANDS):
            pieces.append(p[nxt - r0:r1 - r0] + parts[j + 1][:r1 - nxt])
            cur = r1
    return jnp.concatenate(pieces, axis=0)


def _ln0(x):
    m = jnp.mean(x, axis=0, keepdims=True)
    xc = x - m
    v = jnp.mean(xc * xc, axis=0, keepdims=True)
    return xc * jax.lax.rsqrt(v + EPS)


def _phi(t):
    return jnp.where(t > 0, t + 1.0, jnp.exp(jnp.minimum(t, 0.0))) + 1e-6


def _head(idx):
    return sum((idx >= DH * j).astype(jnp.int32) for j in range(1, H))


def _a_side(a11, a12, a21, a22):
    return [a11 + a22, a21 + a22, a11, a22, a11 + a12, a21 - a11, a12 - a22]


def _b_side(b11, b12, b21, b22):
    return [b11 + b22, b11, b12 - b22, b21 - b11, b22, b11 + b12, b21 + b22]


def _combine(m):
    m1, m2, m3, m4, m5, m6, m7 = m
    return m1 + m4 - m5 + m7, m3 + m5, m2 + m4, m1 - m2 + m3 + m6


def _dot(a, b):
    return jnp.dot(a, b, preferred_element_type=f32)


def _kernel(x_hbm, wqkv_hbm, b1_hbm, b2_hbm, wo_hbm, w1_hbm, w2_hbm, o_ref,
            x_v, wqk_v, wv_v, wqkT, wo_v, w1_v, w2_v, b1_v, b2_v,
            a1, w1r, a2, b2_s, pq_s, g_acc, wpT, zbd, b2c, xn_s, sems):
    step = pl.program_id(0)

    def x_copy(i):
        return pltpu.make_async_copy(x_hbm.at[:, pl.ds(i * TM, TM)],
                                     x_v.at[:, pl.ds(i * TM, TM)], sems.at[i])

    wq_copy = pltpu.make_async_copy(wqkv_hbm.at[:, pl.ds(0, WQ)],
                                    wqk_v.at[:, pl.ds(0, WQ)], sems.at[NS])
    wk_copy = pltpu.make_async_copy(wqkv_hbm.at[:, pl.ds(WQ, 2 * D - WQ)],
                                    wqk_v.at[:, pl.ds(WQ, 2 * D - WQ)], sems.at[NS + 7])
    mlp_copies = [pltpu.make_async_copy(w1_hbm, w1_v, sems.at[NS + 1]),
                  pltpu.make_async_copy(b1_hbm, b1_v, sems.at[NS + 2]),
                  pltpu.make_async_copy(b2_hbm, b2_v, sems.at[NS + 3]),
                  pltpu.make_async_copy(w2_hbm, w2_v, sems.at[NS + 6])]
    late_copies = [pltpu.make_async_copy(wqkv_hbm.at[:, pl.ds(2 * D, D)], wv_v, sems.at[NS + 4]),
                   pltpu.make_async_copy(wo_hbm, wo_v, sems.at[NS + 5])]

    @pl.when(step == 0)
    def _():
        wq_copy.start()
        x_copy(0).start()
        wk_copy.start()
        for k in range(1, NS):
            x_copy(k).start()
        for c in mlp_copies + late_copies:
            c.start()
        g_acc[...] = jnp.zeros(g_acc.shape, f32)
        wq_copy.wait()
        wqkT[:WQ, :] = wqk_v[:, :WQ].T
        x_copy(0).wait()
        xn_s[0] = _ln0(x_v[:, :TM].astype(f32)).astype(bf16)
        wk_copy.wait()
        wqkT[WQ:, :] = wqk_v[:, WQ:].T

    @pl.when(step < NS - 1)
    def _():
        col1 = pl.multiple_of((step + 1) * TM, TM)
        pltpu.make_async_copy(x_hbm.at[:, pl.ds(col1, TM)],
                              x_v.at[:, pl.ds(col1, TM)], sems.at[step + 1]).wait()

    def prep_mlp():
        for c in mlp_copies:
            c.wait()
        for lo in range(0, F2, 128):
            hi = lo + 128
            q = [w1_v[k0:k0 + KM, f0 + lo:f0 + hi].T
                 for f0 in (0, F2) for k0 in (0, KM)]
            for r in range(0, 128, RB):
                for i, t in enumerate(_a_side(*[u[r:r + RB].astype(f32) for u in q])):
                    a1[i, lo + r:lo + r + RB, :] = t.astype(bf16)
        row = jax.lax.broadcasted_iota(jnp.int32, (128 - (D - 2 * KM), F), 0)
        tail = jnp.where(row == 0, jnp.broadcast_to(b1_v[...].reshape(1, F).astype(f32),
                                                    row.shape), 0.0).astype(bf16)
        w1r[...] = jnp.concatenate([w1_v[2 * KM:, :], tail], axis=0).T
        b2c[...] = jnp.broadcast_to(b2_v[...].astype(f32).reshape(1, D), (128, D)).T

    def phase1(prep):
        col0 = pl.multiple_of(step * TM, TM)
        if prep:
            prep_mlp()
        xn = xn_s[step % 2]
        qk = _dot(wqkT[...], xn)
        if not prep:
            col1 = pl.multiple_of((step + 1) * TM, TM)
            xn_s[(step + 1) % 2] = _ln0(x_v[:, pl.ds(col1, TM)].astype(f32)).astype(bf16)
        pq_s[:, pl.ds(col0, TM)] = _phi(qk[:D, :]).astype(bf16)
        pk = _phi(qk[D:, :]).astype(bf16)
        xe = jnp.concatenate([xn, jnp.ones((DP - D, TM), bf16)], axis=0)
        g_acc[...] += jax.lax.dot_general(pk, xe, NT, preferred_element_type=f32)

    @pl.when(step < NS - 1)
    def _():
        phase1(False)

    @pl.when(step == NS - 1)
    def _():
        phase1(True)

    @pl.when(step == NS - 1)
    def _():
        for c in late_copies:
            c.wait()
        wp_parts = []
        for (lo, hi, r0, r1) in BANDS:
            g = g_acc[r0:r1, :]
            kv = _dot(g[:, :D].astype(bf16), wv_v[:, lo:hi])
            r = jax.lax.broadcasted_iota(jnp.int32, (r1 - r0, hi - lo), 0) + r0
            c = jax.lax.broadcasted_iota(jnp.int32, (r1 - r0, hi - lo), 1) + lo
            mask = _head(r) == _head(c)
            kvbd = jnp.where(mask, kv, 0.0).astype(bf16)
            wp_parts.append(_dot(kvbd, wo_v[lo:hi, :]))
            zc = g_acc[lo:hi, D:D + 1]
            zrow = jnp.broadcast_to(zc, (hi - lo, r1 - r0)).T
            zbd[r0:r1, lo:hi] = jnp.where(mask, zrow, 0.0).astype(bf16)
        wpT[...] = _band_assemble(wp_parts).T.astype(bf16)
        for r in range(0, D2, RB):
            for lo in range(0, F2, 256):
                hi = lo + 256
                q = [w2_v[r0 + r:r0 + r + RB, f0 + lo:f0 + hi].astype(f32)
                     for r0 in (0, D2) for f0 in (0, F2)]
                sums = _a_side(*q)
                for j, i in enumerate(A2_SLOTS):
                    a2[j, r:r + RB, lo:hi] = sums[i].astype(bf16)

    @pl.when(step >= NS)
    def _():
        col0 = pl.multiple_of((step - NS) * TM, TM)
        x = x_v[:, pl.ds(col0, TM)].astype(f32)
        pq = pq_s[:, pl.ds(col0, TM)]
        den = _band_assemble([_dot(zbd[r0:r1, lo:hi], pq[lo:hi, :])
                              for (lo, hi, r0, r1) in BANDS]) + 1e-6
        pqn = (pq.astype(f32) / den).astype(bf16)
        h = x + _dot(wpT[...], pqn)
        hn = _ln0(h)
        b1s = [t.astype(bf16) for t in _b_side(hn[:KM, :N2], hn[:KM, N2:],
                                               hn[KM:2 * KM, :N2], hn[KM:2 * KM, N2:])]
        hr = jnp.concatenate([hn[2 * KM:, :].astype(bf16),
                              jnp.ones((128 - (D - 2 * KM), TM), bf16)], axis=0)

        def mm1(c):
            lo, hi = c * FC, (c + 1) * FC
            return ([_dot(a1[i, lo:hi, :], b1s[i]) for i in range(7)],
                    _dot(w1r[lo:hi, :], hr), _dot(w1r[F2 + lo:F2 + hi, :], hr))

        p = None
        nxt = mm1(0)
        for c in range(NFC):
            lo, hi = c * FC, (c + 1) * FC
            ms, rt, rb = nxt
            if c + 1 < NFC:
                nxt = mm1(c + 1)
            for r in range(0, FC, RB):
                c11, c12, c21, c22 = _combine([m[r:r + RB] for m in ms])
                acts = []
                for t in (c11 + rt[r:r + RB, :N2], c12 + rt[r:r + RB, N2:],
                          c21 + rb[r:r + RB, :N2], c22 + rb[r:r + RB, N2:]):
                    t = jnp.maximum(t, 0.0)
                    acts.append(t * t)
                for i, t in enumerate(_b_side(*acts)):
                    b2_s[i, lo + r:lo + r + RB, :] = t.astype(bf16)
            lhs = {i: a2[j, :, lo:hi] for j, i in enumerate(A2_SLOTS)}
            lhs[2] = w2_v[:D2, lo:hi]
            lhs[3] = w2_v[D2:, F2 + lo:F2 + hi]
            pc = [_dot(lhs[i], b2_s[i, lo:hi, :]) for i in range(7)]
            p = pc if p is None else [u + v for u, v in zip(p, pc)]
        o11, o12, o21, o22 = _combine(p)
        mlp = jnp.concatenate([jnp.concatenate([o11, o12], axis=1),
                               jnp.concatenate([o21, o22], axis=1)], axis=0)
        out = h + mlp + jnp.concatenate([b2c[...]] * (TM // 128), axis=1)
        o_ref[...] = out.astype(o_ref.dtype)


@jax.jit
def pallas_sequential_preLN__linear_attn_block__dense_activation_squared_relu__prompt_kernel(
    A_x, A_wqkv, A_wo, B_x, B_w1, B_b1, B_w2, B_b2):
    xT = jnp.swapaxes(A_x, 1, 2).reshape(D, S)
    w2T = B_w2.T
    out = pl.pallas_call(
        _kernel,
        grid=(2 * NS,),
        in_specs=[pl.BlockSpec(memory_space=pl.ANY)] * 7,
        out_specs=pl.BlockSpec((D, TM), lambda i: (0, jnp.maximum(i - NS, 0))),
        out_shape=jax.ShapeDtypeStruct((D, S), bf16),
        scratch_shapes=[
            pltpu.VMEM((D, S), bf16),
            pltpu.VMEM((D, 2 * D), bf16),
            pltpu.VMEM((D, D), bf16),
            pltpu.VMEM((2 * D, D), bf16),
            pltpu.VMEM((D, D), bf16),
            pltpu.VMEM((D, F), bf16),
            pltpu.VMEM((D, F), bf16),
            pltpu.VMEM((F,), bf16),
            pltpu.VMEM((D,), bf16),
            pltpu.VMEM((7, F2, KM), bf16),
            pltpu.VMEM((F, 128), bf16),
            pltpu.VMEM((5, D2, F2), bf16),
            pltpu.VMEM((7, F2, N2), bf16),
            pltpu.VMEM((D, S), bf16),
            pltpu.VMEM((D, DP), f32),
            pltpu.VMEM((D, D), bf16),
            pltpu.VMEM((D, D), bf16),
            pltpu.VMEM((D, 128), f32),
            pltpu.VMEM((2, D, TM), bf16),
            pltpu.SemaphoreType.DMA((NS + 8,)),
        ],
        compiler_params=pltpu.CompilerParams(
            dimension_semantics=("arbitrary",),
            vmem_limit_bytes=100 * 1024 * 1024),
    )(xT, A_wqkv, B_b1, B_b2, A_wo, B_w1, w2T)
    return jnp.swapaxes(out.reshape(1, D, S), 1, 2)
```
